```python
import os as _os
_os.environ.setdefault("JAX_PLATFORMS", "cpu")
import jax
import jax.numpy as jnp

def _softmax(x, axis=-1):
    return jax.nn.softmax(x, axis=axis)
def _gelu(x):
    return jax.nn.gelu(x, approximate=True)
def _silu(x):
    return jax.nn.silu(x)
def _sigmoid(x):
    return jax.nn.sigmoid(x)
def _layernorm(x, axis=-1, eps=1e-5):
    m = jnp.mean(x, axis=axis, keepdims=True)
    v = jnp.var(x, axis=axis, keepdims=True)
    return (x - m) / jnp.sqrt(v + eps)
def _scatter_add(tgt, idx, src, axis=0):
    return tgt.at[idx].add(src)
def _segment_sum(src, seg, n):
    return jax.ops.segment_sum(src, seg, n)
class _Rng:
    def __init__(self, key):
        self._k = key
    def _next(self):
        self._k, sub = jax.random.split(self._k)
        return sub
    def normal(self, shape):
        return jax.random.normal(self._next(), shape, dtype=jnp.bfloat16)
    def randint(self, lo, hi, shape):
        return jax.random.randint(self._next(), shape, lo, hi, dtype=jnp.int32)
    def uniform(self, shape, lo=0.0, hi=1.0):
        return jax.random.uniform(self._next(), shape, jnp.bfloat16, lo, hi)
    def permutation(self, n):
        return jax.random.permutation(self._next(), n)


kernel_name = 'interleave_layers__sliding_local_dilated__moe_arch_mod__prompt'

def setup_inputs():
    _rng = _Rng(jax.random.key(int.from_bytes(__import__("os").urandom(4), "little")))
    _w = (lambda a: (lambda t: t.astype(jnp.bfloat16) if jnp.issubdtype(t.dtype, jnp.floating) else t)(jnp.asarray(a)))
    def _A_setup():
        B, S, D = 1, 2048, 512
        return {
            "x": _w((lambda *s: _rng.normal(s) * 0.05)(B, S, D)),
            "wqkv": _w((lambda *s: _rng.normal(s) * 0.05)(D, 3 * D)),
            "wo": _w((lambda *s: _rng.normal(s) * 0.05)(D, D)),
        }
    _A_in = _A_setup()

    def _B_setup():
        B, S, D, F, C = 1, 2048, 512, 1376, 2
        return {
            "x": _w((lambda *s: _rng.normal(s) * 0.05)(B, S, D)),
            "w_r": _w((lambda *s: _rng.normal(s) * 0.05)(D)),
            "w_gate": _w((lambda *s: _rng.normal(s) * 0.05)(D, F)),
            "w_up": _w((lambda *s: _rng.normal(s) * 0.05)(D, F)),
            "w_down": _w((lambda *s: _rng.normal(s) * 0.05)(F, D)),
        }
    _B_in = _B_setup()

    return {
        "A_x": _A_in["x"],
        "A_wqkv": _A_in["wqkv"],
        "A_wo": _A_in["wo"],
        "B_x": _B_in["x"],
        "B_w_r": _B_in["w_r"],
        "B_w_gate": _B_in["w_gate"],
        "B_w_up": _B_in["w_up"],
        "B_w_down": _B_in["w_down"],
    }

def reference(A_x, A_wqkv, A_wo, B_x, B_w_r, B_w_gate, B_w_up, B_w_down):
    def _A_ref(x, wqkv, wo):
        B, S, D = x.shape
        H = 32; Dh = D // H
        W, dil = 8, 2
        qkv = (lambda x, *d: x.transpose(*d))((x @ wqkv).reshape(B, S, 3, H, Dh), 2, 0, 3, 1, 4)
        q, k, v = qkv[0], qkv[1], qkv[2]
        scale = Dh ** -0.5
        pos = jnp.arange(S)
        off = jnp.arange(W) * dil
        idx = pos[:, None] - off[None, :]
        mask = idx >= 0
        idx_c = jnp.where(mask, idx, 0).reshape(-1)
        kg = k[:, :, idx_c, :].reshape(B, H, S, W, Dh)
        vg = v[:, :, idx_c, :].reshape(B, H, S, W, Dh)
        logits = jnp.einsum("bhsd,bhswd->bhsw", q, kg) * scale
        logits = jnp.where(mask[None, None, :, :], logits, -1e9)
        attn = _softmax(logits, axis=-1)
        o = jnp.einsum("bhsw,bhswd->bhsd", attn, vg)
        return (lambda x, *d: x.transpose(*d))(o, 0, 2, 1, 3).reshape(B, S, D) @ wo

    def _B_ref(x, w_r, w_gate, w_up, w_down):
        B, S, D = x.shape
        C = 2
        r = x @ w_r
        idx = jnp.argsort(-r, axis=-1)[:, :C]
        idx_e = jnp.repeat(idx.reshape(B, C, 1), D, axis=2)
        x_sel = jnp.take_along_axis(x, idx_e, axis=1)
        g = _silu(x_sel @ w_gate)
        u = x_sel @ w_up
        y = (g * u) @ w_down
        r_sel = _sigmoid(jnp.take_along_axis(r, idx, axis=1))
        y = y * r_sel.reshape(B, C, 1)
        b_off = (jnp.arange(B) * S).reshape(B, 1)
        flat_idx = (idx + b_off).reshape(B * C)
        zero = (x * 0.0).reshape(B * S, D)
        upd = _scatter_add(zero, flat_idx, y.reshape(B * C, D), axis=0)
        return x + upd.reshape(B, S, D)

    x = A_x
    x = x + _A_ref(_layernorm(x, axis=-1), A_wqkv, A_wo)
    x = x + _B_ref(_layernorm(x, axis=-1), B_w_r, B_w_gate, B_w_up, B_w_down)
    x = x + _A_ref(_layernorm(x, axis=-1), A_wqkv, A_wo)
    x = x + _B_ref(_layernorm(x, axis=-1), B_w_r, B_w_gate, B_w_up, B_w_down)
    return x
```

```python
import functools
import math

import jax
import jax.numpy as jnp
import numpy as np
from jax import lax
import jax.experimental.pallas as pl
import jax.experimental.pallas.tpu as pltpu

S = 2048
D = 512
F = 1376
NW = 8
DIL = 2
HALO = 16
EPS = 1e-5
LOG2E = math.log2(math.e)
SCALE = 0.25

f32 = jnp.float32
bf16 = jnp.bfloat16
i32 = jnp.int32


def _make_kernel(TB, R, RL):
    NB = S // TB
    assert NB % 2 == 0 and NB >= 4

    def kernel(x_hbm, wqkv_hbm, wo_hbm, wr_ref, wg_hbm, wu_hbm, wd_hbm, out_hbm,
               xin, wqkv_v, wo_v, wg_v, wu_v, wd_v,
               t_s, wof_s, wp, wop,
               q0, q1, k0, k1, v0, v1, o0, o1, ln0, ln1,
               xa, xb, outv, r_s, patch,
               sem_x, sem_w, sem_o, sem_p):
        qb, kb, vb, ob, lnb = (q0, q1), (k0, k1), (v0, v1), (o0, o1), (ln0, ln1)

        def x_copy(b):
            return pltpu.make_async_copy(x_hbm.at[0, pl.ds(b * TB, TB), :],
                                         xin.at[pl.ds(b * TB, TB), :], sem_x.at[b])

        def wqkv_copy(m):
            return pltpu.make_async_copy(wqkv_hbm.at[:, pl.ds(m * D, D)],
                                         wqkv_v.at[:, pl.ds(m * D, D)], sem_w.at[m])

        wo_copy = pltpu.make_async_copy(wo_hbm, wo_v, sem_w.at[3])
        wg_copy = pltpu.make_async_copy(wg_hbm, wg_v, sem_w.at[4])
        wu_copy = pltpu.make_async_copy(wu_hbm, wu_v, sem_w.at[5])
        wd_copy = pltpu.make_async_copy(wd_hbm, wd_v, sem_w.at[6])

        def out_copy(b):
            return pltpu.make_async_copy(outv.at[pl.ds(b * TB, TB), :],
                                         out_hbm.at[0, pl.ds(b * TB, TB), :], sem_o.at[b])

        wqkv_copy(0).start()
        x_copy(0).start()
        wqkv_copy(1).start()
        wqkv_copy(2).start()
        x_copy(1).start()
        wo_copy.start()
        for b in range(2, NB):
            x_copy(b).start()
        wg_copy.start()
        wu_copy.start()
        wd_copy.start()

        def prep_qkv(m):
            for i in range(4):
                u = pltpu.bitcast(wqkv_v[:, pl.ds(m * D + i * 128, 128)], i32)
                ut = u.T
                t_s[0, pl.ds(i * 128, 128), :] = ut[:, :128]
                t_s[1, pl.ds(i * 128, 128), :] = ut[:, 128:]
            for j in range(4):
                for kp in range(2):
                    rows = jnp.concatenate(
                        [t_s[kp, pl.ds(4 * j + g, 32, stride=16), :] for g in range(4)], axis=0)
                    wp[m * 4 + j, pl.ds(kp * 256, 256), :] = pltpu.bitcast(rows.T, bf16)

        def prep_wo():
            for j in range(4):
                wof_s[j] = wo_v[:, pl.ds(j * 128, 128)].astype(f32)
            for j in range(4):
                for d in range(16):
                    wop[j, pl.ds(d * 32, 32), :] = wof_s[j, pl.ds(d, 32, stride=16), :].astype(bf16)

        lane = lax.broadcasted_iota(i32, (R, 128), 1)
        grp = lane >> 5
        m_lo = lane < 64
        m_mid = (grp == 1) | (grp == 2)
        m_even = (grp & 1) == 0

        def layernorm(x):
            mu = jnp.sum(x, axis=-1, keepdims=True) * (1.0 / D)
            xc = x - mu
            var = jnp.sum(xc * xc, axis=-1, keepdims=True) * (1.0 / D)
            return xc * lax.rsqrt(var + EPS)

        def load_x(layer, row0, n):
            if layer == 0:
                return xin[pl.ds(row0, n), :].astype(f32)
            return xa[pl.ds(row0, n), :]

        def stage_a_ln(layer, blk, p):
            row0 = pl.multiple_of(blk * TB, TB)
            for c in range(TB // RL):
                ln = layernorm(load_x(layer, row0 + c * RL, RL)).astype(bf16)
                for j in range(4):
                    lnb[p][j, pl.ds(c * RL, RL), :] = ln[:, j * 128:(j + 1) * 128]

        def stage_a_mm(p, m):
            lhs = jnp.concatenate([lnb[p][j] for j in range(4)], axis=1)
            rhs = jnp.concatenate([wp[m * 4 + j] for j in range(4)], axis=1)
            res = jnp.dot(lhs, rhs, preferred_element_type=f32)
            for j in range(4):
                if m == 0:
                    qb[p][j] = res[:, j * 128:(j + 1) * 128]
                else:
                    (kb, vb)[m - 1][p][j, pl.ds(HALO, TB), :] = res[:, j * 128:(j + 1) * 128]

        def stage_a(layer, blk, p):
            stage_a_ln(layer, blk, p)
            for m in range(3):
                stage_a_mm(p, m)

        def halo_first(p):
            for j in range(4):
                kb[p][j, pl.ds(0, HALO), :] = jnp.broadcast_to(kb[p][j, pl.ds(HALO, 1), :], (HALO, 128))
                vb[p][j, pl.ds(0, HALO), :] = jnp.broadcast_to(vb[p][j, pl.ds(HALO, 1), :], (HALO, 128))

        def halo_next(p):
            for j in range(4):
                kb[1 - p][j, pl.ds(0, HALO), :] = kb[p][j, pl.ds(TB, HALO), :]
                vb[1 - p][j, pl.ds(0, HALO), :] = vb[p][j, pl.ds(TB, HALO), :]

        def combine4(a, b, c, d):
            qa = jnp.where(m_lo, a, b) + pltpu.roll(jnp.where(m_lo, b, a), 64, 1)
            qc = jnp.where(m_mid, c, d) + pltpu.roll(jnp.where(m_mid, d, c), 64, 1)
            return jnp.where(m_even, qa, qc) + pltpu.roll(jnp.where(m_even, qc, qa), 96, 1)

        def spread4(e):
            t = pltpu.roll(e, 32, 1)
            u0 = jnp.where(m_even, e, t)
            u1 = jnp.where(m_even, t, e)
            r0 = pltpu.roll(u0, 64, 1)
            r1 = pltpu.roll(u1, 64, 1)
            return (jnp.where(m_lo, u0, r0), jnp.where(m_lo, r0, u0),
                    jnp.where(m_mid, u1, r1), jnp.where(m_mid, r1, u1))

        def stage_b(p, first):
            for c in range(TB // R):
                t0 = c * R
                qs = [qb[p][j, pl.ds(t0, R), :] for j in range(4)]
                ps = []
                for w in range(NW):
                    acc = None
                    for j in range(4):
                        t = qs[j] * kb[p][j, pl.ds(HALO + t0 - DIL * w, R), :]
                        acc = t if acc is None else acc + t
                    ps.append(acc)
                la = combine4(*ps[:4])
                lb = combine4(*ps[4:])
                if first and t0 < HALO:
                    pos = lax.broadcasted_iota(i32, (R, 128), 0) + t0
                    wa = ((grp & 1) << 1) | (grp >> 1)
                    la = jnp.where(pos >= DIL * wa, la, -1e9 / SCALE)
                    lb = jnp.where(pos >= DIL * (wa + 4), lb, -1e9 / SCALE)
                m = jnp.maximum(la, lb)
                m = jnp.maximum(m, pltpu.roll(m, 64, 1))
                m = jnp.maximum(m, pltpu.roll(m, 32, 1))
                ea = jnp.exp2((la - m) * (SCALE * LOG2E))
                eb = jnp.exp2((lb - m) * (SCALE * LOG2E))
                s = ea + eb
                s = s + pltpu.roll(s, 64, 1)
                s = s + pltpu.roll(s, 32, 1)
                inv = 1.0 / s
                pw = spread4(ea * inv) + spread4(eb * inv)
                for j in range(4):
                    acc = None
                    for w in range(NW):
                        t = pw[w] * vb[p][j, pl.ds(HALO + t0 - DIL * w, R), :]
                        acc = t if acc is None else acc + t
                    ob[p][j, pl.ds(t0, R), :] = acc.astype(bf16)

        def stage_c(layer, blk, p):
            row0 = pl.multiple_of(blk * TB, TB)
            wr = wr_ref[...].astype(f32).reshape(1, D)
            lhs = jnp.concatenate([ob[p][j] for j in range(4)], axis=1)
            rhs = jnp.concatenate([wop[j] for j in range(4)], axis=1)
            y = jnp.dot(lhs, rhs, preferred_element_type=f32)
            lane8 = lax.broadcasted_iota(i32, (8, 128), 1)
            racc = jnp.full((8, 128), -jnp.inf, f32)
            for c in range(TB // RL):
                rows = pl.ds(row0 + c * RL, RL)
                x1 = load_x(layer, row0 + c * RL, RL) + y[c * RL:(c + 1) * RL]
                ln = layernorm(x1)
                r = jnp.sum(ln * wr, axis=-1, keepdims=True)
                for g in range(RL // 8):
                    racc = jnp.where(lane8 == c * (RL // 8) + g, r[g * 8:(g + 1) * 8], racc)
                xb[rows, :] = x1
                if layer == 0:
                    xa[rows, :] = x1 + ln
                else:
                    outv[rows, :] = (x1 + ln).astype(bf16)
            r_s[blk] = racc
            if layer == 1:
                out_copy(blk).start()

        def run_layer(layer):
            if layer == 0:
                wqkv_copy(0).wait()
                prep_qkv(0)
                x_copy(0).wait()
                stage_a_ln(0, 0, 0)
                wqkv_copy(1).wait()
                stage_a_mm(0, 0)
                prep_qkv(1)
                wqkv_copy(2).wait()
                stage_a_mm(0, 1)
                prep_qkv(2)
                stage_a_mm(0, 2)
                x_copy(1).wait()
                wo_copy.wait()
                prep_wo()
            else:
                stage_a(layer, 0, 0)
            halo_first(0)
            halo_next(0)
            stage_a(layer, 1, 1)
            stage_b(0, True)

            def body(it, carry):
                for p in (1, 0):
                    i = 2 * it + 2 - p
                    if layer == 0:
                        x_copy(i + 1).wait()
                    halo_next(p)
                    stage_a(layer, i + 1, 1 - p)
                    stage_b(p, False)
                    stage_c(layer, i - 1, 1 - p)
                return carry

            lax.fori_loop(0, (NB - 2) // 2, body, 0)
            stage_b(1, False)
            stage_c(layer, NB - 2, 0)
            stage_c(layer, NB - 1, 1)

        def route_and_ffn():
            rr = r_s[...].reshape(NB * 8, 128)
            row = lax.broadcasted_iota(i32, (NB * 8, 128), 0)
            col = lax.broadcasted_iota(i32, (NB * 8, 128), 1)
            tok = jnp.where(col < TB // 8, (row >> 3) * TB + col * 8 + (row & 7), S)
            key = jnp.where(rr != rr, -jnp.inf, rr)
            m1 = jnp.max(key)
            i1 = jnp.min(jnp.where(key == m1, tok, S))
            rest = tok != i1
            key2 = jnp.where(rest, key, -jnp.inf)
            m2 = jnp.max(key2)
            i2 = jnp.min(jnp.where((key2 == m2) & rest, tok, S))
            i1 = jnp.clip(i1, 0, S - 1)
            i2 = jnp.clip(i2, 0, S - 1)
            sub = lax.broadcasted_iota(i32, (16, D), 0)
            xs = jnp.where(sub == 0, xb[pl.ds(i1, 1), :], xb[pl.ds(i2, 1), :])
            lns = layernorm(xs)
            wr = wr_ref[...].astype(f32).reshape(1, D)
            gate = jax.nn.sigmoid(jnp.sum(lns * wr, axis=-1, keepdims=True))
            lnq = lns.astype(bf16)
            g = lax.dot_general(lnq, wg_v[...], (((1,), (1,)), ((), ())), preferred_element_type=f32)
            u = lax.dot_general(lnq, wu_v[...], (((1,), (1,)), ((), ())), preferred_element_type=f32)
            h = (g * jax.nn.sigmoid(g) * u).astype(bf16)
            y = jnp.dot(h, wd_v[...], preferred_element_type=f32)
            return i1, i2, xs + (lns + y * gate)

        run_layer(0)
        wg_copy.wait()
        wu_copy.wait()
        wd_copy.wait()
        i1, i2, new = route_and_ffn()
        xa[pl.ds(i1, 1), :] = new[0:1]
        xa[pl.ds(i2, 1), :] = new[1:2]

        run_layer(1)
        i1, i2, new = route_and_ffn()
        b1 = pl.multiple_of((i1 >> 4) << 4, 16)
        b2 = pl.multiple_of((i2 >> 4) << 4, 16)
        sub = lax.broadcasted_iota(i32, (16, D), 0)
        for n, b in enumerate((b1, b2)):
            t = outv[pl.ds(b, 16), :].astype(f32)
            t = jnp.where(sub + b == i1, new[0:1], t)
            t = jnp.where(sub + b == i2, new[1:2], t)
            patch[n] = t.astype(bf16)
        for b in range(NB):
            out_copy(b).wait()
        c1 = pltpu.make_async_copy(patch.at[0], out_hbm.at[0, pl.ds(b1, 16), :], sem_p.at[0])
        c2 = pltpu.make_async_copy(patch.at[1], out_hbm.at[0, pl.ds(b2, 16), :], sem_p.at[1])
        c1.start()

        @pl.when(b1 != b2)
        def _():
            c2.start()
            c2.wait()

        c1.wait()

    V = pltpu.VMEM
    scratch = [
        V((S, D), bf16), V((D, 3 * D), bf16), V((D, D), bf16),
        V((F, D), bf16), V((F, D), bf16), V((F, D), bf16),
        V((2, D, 128), i32), V((4, D, 128), f32), V((12, D, 128), bf16), V((4, D, 128), bf16),
        V((4, TB, 128), f32), V((4, TB, 128), f32),
        V((4, TB + HALO, 128), f32), V((4, TB + HALO, 128), f32),
        V((4, TB + HALO, 128), f32), V((4, TB + HALO, 128), f32),
        V((4, TB, 128), bf16), V((4, TB, 128), bf16),
        V((4, TB, 128), bf16), V((4, TB, 128), bf16),
        V((S, D), f32), V((S, D), f32), V((S, D), bf16), V((NB, 8, 128), f32), V((2, 16, D), bf16),
        pltpu.SemaphoreType.DMA((NB,)), pltpu.SemaphoreType.DMA((7,)),
        pltpu.SemaphoreType.DMA((NB,)), pltpu.SemaphoreType.DMA((2,)),
    ]
    return kernel, scratch


def build(TB=256, R=16, RL=32, flags=None):
    kernel, scratch = _make_kernel(TB, R, RL)

    def fn(A_x, A_wqkv, A_wo, B_x, B_w_r, B_w_gate, B_w_up, B_w_down):
        del B_x
        any_spec = pl.BlockSpec(memory_space=pltpu.HBM)
        hbm = lambda a: pltpu.with_memory_space_constraint(a, pltpu.HBM)
        return pl.pallas_call(
            kernel,
            out_shape=jax.ShapeDtypeStruct((1, S, D), bf16),
            in_specs=[any_spec, any_spec, any_spec, pl.BlockSpec(memory_space=pltpu.VMEM),
                      any_spec, any_spec, any_spec],
            out_specs=any_spec,
            scratch_shapes=scratch,
            compiler_params=pltpu.CompilerParams(vmem_limit_bytes=100 * 1024 * 1024, disable_bounds_checks=True, flags=flags),
            name="fused",
        )(hbm(A_x), hbm(A_wqkv), hbm(A_wo), hbm(B_w_r), hbm(B_w_gate.T), hbm(B_w_up.T), hbm(B_w_down))

    return fn


_fused = build(TB=256,R=64,RL=64)


@jax.jit
def pallas_interleave_layers__sliding_local_dilated__moe_arch_mod__prompt_kernel(
    A_x: jax.Array,
    A_wqkv: jax.Array,
    A_wo: jax.Array,
    B_x: jax.Array,
    B_w_r: jax.Array,
    B_w_gate: jax.Array,
    B_w_up: jax.Array,
    B_w_down: jax.Array,
):
    return _fused(A_x, A_wqkv, A_wo, B_x, B_w_r, B_w_gate, B_w_up, B_w_down)
```

```python
import math

import jax
import jax.numpy as jnp
from jax import lax
import jax.experimental.pallas as pl
import jax.experimental.pallas.tpu as pltpu

S = 2048
D = 512
F = 1376
NW = 8
HALO = 8
EPS = 1e-5
LOG2E = math.log2(math.e)
QSCALE = 0.25 * LOG2E
TB = 256
HB = TB // 2
NB = S // TB
P = S // 2
RL = 16
NS = 2
FT = [min(n * 128, F - 128) for n in range(-(-F // 128))]

LN2_0, ATT_0, LN1_0, WO_0, WF_0 = 0, S, 2 * S, 3 * S, 3 * S + D

f32 = jnp.float32
bf16 = jnp.bfloat16
i32 = jnp.int32


def _emit(tasks):
    pending = sorted(enumerate(tasks), key=lambda t: (t[1][0], t[0]))
    active = []
    tick = pending[0][1][0]
    while pending or active:
        while pending and pending[0][1][0] <= tick:
            active.append(pending.pop(0)[1][1])
        alive = []
        for g in active:
            try:
                next(g)
                alive.append(g)
            except StopIteration:
                pass
        active = alive
        tick += 1


def _once(fn, *args):
    fn(*args)
    return
    yield


def _tree(op, xs):
    while len(xs) > 1:
        xs = [op(xs[i], xs[i + 1]) for i in range(0, len(xs), 2)]
    return xs[0]


def _half(words, e):
    return lax.bitcast_convert_type(words << 16 if e == 0 else words & -65536, f32)


def _words(even, odd):
    lo, hi = (lax.bitcast_convert_type(v.astype(bf16).astype(f32), i32) for v in (even, odd))
    return lax.shift_right_logical(lo, 16) | hi


def _tile(x, j):
    return x[:, j * 128:(j + 1) * 128]


def _rowsum(x):
    return jnp.sum(x, axis=-1, keepdims=True)


def _start(copies):
    for c in copies:
        c.start()


def _kernel(x_hbm, wqkv_hbm, wo_hbm, wr_hbm, wg_hbm, wu_hbm, wd_hbm, out_hbm,
            xin, wqkv_v, wo_v, wr_v, wg_v, wu_v, wd_v,
            t_s, wof_s, wp, wr_s,
            q_s, k_s, v_s, xa, xb, outv, r_s, patch,
            sem_in, sem_out, ops, *ln2_early):
    xin_w, out_w, patch_w, ops_w = (r.bitcast(i32) for r in (xin, outv, patch, ops))

    def ln_buf(layer, blk):
        if layer == 0:
            return ops, LN1_0 + blk * TB
        return (ln2_early[blk], 0) if blk < NS else (ops, LN2_0 + (blk - NS) * TB)

    def x_copies(b0, b1, sem):
        rows = pl.ds(b0 * TB, (b1 - b0) * TB)
        return [pltpu.make_async_copy(x_hbm.at[0, rows, pl.ds(j * 128, 128)], xin.at[j, rows, :],
                                      sem_in.at[sem]) for j in range(4)]

    def out_copies(b):
        rows = pl.ds(b * TB, TB)
        return [pltpu.make_async_copy(outv.at[j, rows, :], out_hbm.at[0, rows, pl.ds(j * 128, 128)],
                                      sem_out.at[int(b >= NB - 2)]) for j in range(4)]

    def wqkv_copy(m, r0, n, sem):
        return [pltpu.make_async_copy(wqkv_hbm.at[pl.ds(r0, n), pl.ds(m * D, D)],
                                      wqkv_v.at[pl.ds(r0, n), pl.ds(m * D, D)], sem_in.at[sem])]

    XS = NB - 2
    g_x0 = x_copies(0, 1, 0)
    g_qa = wqkv_copy(0, 0, D // 2, 1)
    g_qb = wqkv_copy(0, D // 2, D // 2, 2)
    g_x1 = x_copies(1, 2, 3)
    g_k = wqkv_copy(1, 0, D, 4)
    g_v = wqkv_copy(2, 0, D, 5)
    g_o = [pltpu.make_async_copy(wo_hbm, wo_v, sem_in.at[6]),
           pltpu.make_async_copy(wr_hbm, wr_v, sem_in.at[6])] + x_copies(2, XS, 6)
    g_f = x_copies(XS, NB, 7) + [pltpu.make_async_copy(wg_hbm, wg_v, sem_in.at[7]),
                                 pltpu.make_async_copy(wu_hbm, wu_v, sem_in.at[7]),
                                 pltpu.make_async_copy(wd_hbm, wd_v, sem_in.at[7])]

    due, fine, hold = [], [], [0]

    def wait(copies):
        hold[0] = 3
        for c in copies:
            c.wait()

    def deadline(v, lag):
        for _ in range(lag):
            yield
        due.append(_tree(jnp.maximum, [v[r:r + 8] for r in range(0, v.shape[0], 8)]))

    def rhs_of(w):
        hold[0] -= 1
        if due and hold[0] < 0:
            y = due[0]
            for z in due[1:]:
                y = jnp.maximum(y, z)
            del due[:]
            mid = jnp.where(y < -jnp.inf, jnp.zeros_like(w[56:64]), w[56:64])
            w = jnp.concatenate([w[:56], mid, w[64:]], axis=0)
        return pltpu.bitcast(w, bf16)

    def settle(res):
        if not fine:
            return res
        parts = [res[r:r + 8] for r in range(0, res.shape[0], 8)]
        for c, y in enumerate(fine):
            g = (c * len(parts)) // len(fine)
            parts[g] = jnp.where(y < -jnp.inf, y, parts[g])
        del fine[:]
        return jnp.concatenate(parts, axis=0)

    def lhs_of(ref, spans):
        words = ref.bitcast(i32)
        return jnp.concatenate(
            [pltpu.bitcast(jnp.concatenate([words[kk, pl.ds(r0 // 2, n // 2), :] for r0, n in spans],
                                           axis=0), bf16) for kk in range(4)], axis=1)

    def prep_qkv(m, kp):
        for i in range(4):
            u = pltpu.bitcast(wqkv_v[pl.ds(kp * 256, 256), pl.ds(m * D + i * 128, 128)], i32)
            t_s[kp, pl.ds(i * 128, 128), :] = u.T
        yield
        for j in range(4):
            rows = jnp.concatenate(
                [t_s[kp, pl.ds(4 * j + g, 32, stride=16), :] for g in range(4)], axis=0)
            wp[m * 4 + j, pl.ds(kp * 128, 128), :] = rows.T

    def prep_wr():
        wr_s[...] = jnp.broadcast_to(wr_v[...].astype(f32).reshape(1, D), (8, D))

    def prep_wo(j):
        wof_s[j, pl.ds(0, D), :] = wo_v[:, pl.ds(j * 128, 128)].astype(f32)
        for d in range(16):
            t = wof_s[j, pl.ds(d, 32, stride=16), :]
            ops[j, pl.ds(WO_0 + d * 32, 32), :] = t.astype(bf16)
            if d % 4 == 3:
                fine.append(t[:8])
                yield

    def prep_ffn(n):
        t = (wg_v, wu_v)[n % 2][pl.ds(FT[n // 2], 128), :].astype(f32).T
        ops[n % 4, pl.ds(WF_0 + (n // 4) * D, D), :] = t.astype(bf16)
        yield from deadline(t[D - 8:], 2)

    def ffn_weight(n):
        return pltpu.bitcast(ops_w[n % 4, pl.ds((WF_0 + (n // 4) * D) // 2, D // 2), :], bf16)

    def ln_a(e, p0):
        x = jnp.concatenate([_half(xin_w[j, pl.ds(p0, RL), :], e) for j in range(4)], axis=1)
        s1 = _rowsum(x)
        yield
        xc = x - s1 * (1.0 / D)
        s2 = _rowsum(xc * xc)
        yield
        rstd = lax.rsqrt(s2 * (1.0 / D) + EPS)
        ln = xc * rstd
        ref, r0 = ln_buf(0, p0 // HB)
        for j in range(4):
            ref[j, pl.ds(r0 + e * HB + p0 % HB, RL), :] = _tile(ln, j).astype(bf16)
        yield from deadline(jnp.broadcast_to(rstd, (RL, 128)), 2)

    def mm_a(layer, blk, m):
        ref, r0 = ln_buf(layer, blk)
        for j in range(4):
            res = jnp.dot(lhs_of(ref, [(r0 + e * HB, HB) for e in range(2)]), rhs_of(wp[m * 4 + j]),
                          preferred_element_type=f32)
            if m == 0:
                res = res * QSCALE
            res = settle(res)
            for e in range(2):
                (q_s, k_s, v_s)[m][e, j, pl.ds(HALO + blk * HB, HB), :] = res[e * HB:(e + 1) * HB]
                yield

    def halo(ref, e):
        for j in range(4):
            ref[e, j, pl.ds(0, HALO), :] = jnp.broadcast_to(ref[0, j, pl.ds(HALO, 1), :], (HALO, 128))

    def attn(e, p0, lag):
        def rows(ref, j, w):
            return ref[e, j, pl.ds(HALO + p0 - w, RL), :]

        if p0 == 0:
            halo(k_s, e)
        qs = [rows(q_s, j, 0) for j in range(4)]
        ls = [_tree(jnp.add, [qs[j] * rows(k_s, j, w) for j in range(4)]) for w in range(NW)]
        rs = [pltpu.roll(l, 64, 1) for l in ls]
        yield
        ls = [l + r for l, r in zip(ls, rs)]
        rs = [pltpu.roll(l, 32, 1) for l in ls]
        yield
        ls = [l + r for l, r in zip(ls, rs)]
        if p0 == 0:
            pos = lax.broadcasted_iota(i32, (RL, 128), 0)
            ls = [jnp.where(pos >= w, l, -1e9 * LOG2E) for w, l in enumerate(ls)]
            halo(v_s, e)
        m = _tree(jnp.maximum, ls)
        es = [jnp.exp2(l - m) for l in ls]
        s = _tree(jnp.add, es)
        inv = pltpu.reciprocal(s, approx=True)
        inv = inv * (2.0 - s * inv)
        outs = []
        for j in range(4):
            acc = es[0] * rows(v_s, j, 0)
            for w in range(1, NW):
                acc = acc + es[w] * rows(v_s, j, w)
            outs.append(acc * inv)
            ops[j, pl.ds(ATT_0 + (p0 // HB) * TB + e * HB + p0 % HB, RL), :] = outs[-1].astype(bf16)
        yield from deadline(inv, lag)
        yield
        fine.extend(jnp.maximum(o[:8], o[8:]) for o in outs)

    def mm_c(layer, p0, n):
        r0 = ATT_0 + (p0 // HB) * TB + p0 % HB
        for j in range(4):
            y = jnp.dot(lhs_of(ops, [(r0 + e * HB, n) for e in range(2)]),
                        rhs_of(ops_w[j, pl.ds(WO_0 // 2, D // 2), :]), preferred_element_type=f32)
            y = settle(y)
            cols = pl.ds(j * 128, 128)
            for e in range(2):
                x = _half(xin_w[j, pl.ds(p0, n), :], e) if layer == 0 else xa[e, pl.ds(p0, n), cols]
                xb[e, pl.ds(p0, n), cols] = x + y[e * n:(e + 1) * n]
                if n == HB or e:
                    yield

    def ln_c(layer, parts, racc):
        x = jnp.concatenate([xb[e, pl.ds(p, 8), :] for e, p in parts], axis=0)
        s1 = _rowsum(x)
        yield
        mu = s1 * (1.0 / D)
        xc = x - mu
        s2 = _rowsum(xc * xc)
        s3 = _rowsum(xc * jnp.concatenate([wr_s[...]] * 2, axis=0))
        yield
        var = s2 * (1.0 / D)
        rstd = lax.rsqrt(var + EPS)
        r = s3 * rstd
        lane = lax.broadcasted_iota(i32, (8, 128), 1)
        for g, (e, p) in enumerate(parts):
            racc[e] = jnp.where(lane == p // 8, r[g * 8:(g + 1) * 8], racc[e])
            racc[2] += 1
        if racc[2] == S // 8:
            r_s[0] = racc[0]
            r_s[1] = racc[1]
        gain = 1.0 + rstd
        x2 = xc * gain + mu
        if layer == 0:
            e, p = parts[0]
            xa[e, pl.ds(p, RL), :] = x2
            ln2 = xc * (gain * lax.rsqrt(var * gain * gain + EPS))
            ref, r0 = ln_buf(1, p // HB)
            for j in range(4):
                ref[j, pl.ds(r0 + e * HB + p % HB, RL), :] = _tile(ln2, j).astype(bf16)
        else:
            words = _words(x2[:8], x2[8:])
            for j in range(4):
                out_w[j, pl.ds(parts[0][1], 8), :] = _tile(words, j)
            for g, (e, p) in enumerate(parts):
                xa[e, pl.ds(p, 8), :] = xc[g * 8:(g + 1) * 8]
        yield from deadline(jnp.broadcast_to(r, (RL, 128)), 8)

    def route(layer, st):
        keys = []
        for e in range(2):
            r = r_s[e]
            tok = (lax.broadcasted_iota(i32, (8, 128), 1) * 8
                   + lax.broadcasted_iota(i32, (8, 128), 0)) * 2 + e
            top = pltpu.bitcast(jnp.where(r == 0.0, 0.0, r), i32) >> 13
            rank = jnp.where(r != r, 0, jnp.where(top < 0, -1 - (top & 0x3FFFF), top) + 0x40000)
            keys.append(pltpu.bitcast(0x10000000 + (rank << 11) + (S - 1 - tok), f32))
        sel = []
        for _ in range(2):
            m = jnp.max(jnp.max(jnp.maximum(*keys), axis=0, keepdims=True), axis=1, keepdims=True)
            keys = [jnp.where(k == m, 0.0, k) for k in keys]
            i = S - 1 - (pltpu.bitcast(jnp.broadcast_to(m, (8, 128)), i32)[0, 0] & (S - 1))
            sel.append((i & 1, i >> 1))
            yield
        sub = lax.broadcasted_iota(i32, (8, D), 0)

        def pick(ref):
            return jnp.where(sub == 0, *[ref[e, pl.ds(p, 1), :] for e, p in sel])

        xs = pick(xb)
        if layer == 0:
            s1 = _rowsum(xs)
            yield
            xc = xs - s1 * (1.0 / D)
        else:
            xc = pick(xa)
        s2 = _rowsum(xc * xc)
        s3 = _rowsum(xc * wr_s[...])
        rstd = lax.rsqrt(s2 * (1.0 / D) + EPS)
        st.update(sel=sel, xc=xc, rstd=rstd, base=xs + xc * rstd, gate=jax.nn.sigmoid(s3 * rstd))

    def ffn_up(st):
        xq = jnp.concatenate([st["xc"]] * 2, axis=0).astype(bf16)
        hs = []
        for n, f0 in enumerate(FT):
            g, u = (jnp.dot(xq, ffn_weight(2 * n + c), preferred_element_type=f32)[:8] * st["rstd"]
                    for c in range(2))
            h = g * jax.nn.sigmoid(g) * u
            if f0 != n * 128:
                h = jnp.where(lax.broadcasted_iota(i32, (8, 128), 1) >= n * 128 - f0, h, 0.0)
            hs.append(jnp.concatenate([h, h], axis=0).astype(bf16))
        st["h"] = jnp.concatenate(hs, axis=1)

    def ffn_down(st):
        wd = jnp.concatenate([wd_v[pl.ds(f0, 128), :] for f0 in FT], axis=0)
        y = jnp.dot(st["h"], wd, preferred_element_type=f32)[:8]
        st["new"] = st["base"] + y * st["gate"]

    def patch_rows(st):
        new = st["new"]
        for n, (e, p) in enumerate(st["sel"]):
            xa[e, pl.ds(p, 1), :] = new[n:n + 1]
        s1 = _rowsum(new)
        yield
        xc = new - s1 * (1.0 / D)
        s2 = _rowsum(xc * xc)
        yield
        ln = xc * lax.rsqrt(s2 * (1.0 / D) + EPS)
        st["ln2"] = jnp.concatenate([ln, ln], axis=0).astype(bf16)
        sub = lax.broadcasted_iota(i32, (16, 128), 0)
        for n, (e, p) in enumerate(st["sel"]):
            r = (p // HB - NS) * TB + e * HB + p % HB
            b = pl.multiple_of((jnp.maximum(r, 0) >> 4) << 4, 16)
            for j in range(4):
                t = ops[j, pl.ds(LN2_0 + b, 16), :].astype(f32)
                t = jnp.where(sub + b == r, _tile(ln[n:n + 1], j), t)
                ops[j, pl.ds(LN2_0 + b, 16), :] = t.astype(bf16)

    def patch_qkv(st):
        for m, ref in enumerate((q_s, k_s, v_s)):
            for j in range(4):
                res = jnp.dot(st["ln2"], pltpu.bitcast(wp[m * 4 + j], bf16), preferred_element_type=f32)
                if m == 0:
                    res = res * QSCALE
                for n, (e, p) in enumerate(st["sel"]):
                    ref[e, j, pl.ds(HALO + p, 1), :] = res[n:n + 1]
            yield

    stream, tasks, clock, end = [], [], [0], {}

    def mxu(name, gen, ticks):
        stream.append((clock[0], gen))
        clock[0] += ticks
        end[name] = clock[0]

    def at(tick, fn, *args):
        tasks.append((tick, _once(fn, *args)))

    def spread(first, span, gens):
        for c, g in enumerate(gens):
            tasks.append((first + (c * span) // len(gens), g))

    def proj(layer, b, ms=(0, 1, 2)):
        for m in ms:
            mxu(("A", layer, b, m), mm_a(layer, b, m), 8)

    def out_proj(layer, b):
        mxu(("C", layer, b), mm_c(layer, b * HB, HB), 8)

    st0, st1 = {}, {}
    for b, m in ((0, 0), (1, 0), (0, 1), (0, 2), (1, 1), (1, 2)):
        proj(0, b, (m,))
    done = 0
    for b in range(2, NB):
        proj(0, b)
        while done <= b - (2 if b < 4 else 1):
            out_proj(0, done)
            done += 1
    proj(1, 0, (0, 1))
    out_proj(0, NB - 1)
    proj(1, 0, (2,))
    proj(1, 1, (0,))
    mxu("up", _once(ffn_up, st0), 5)
    proj(1, 1, (1,))
    mxu("down", _once(ffn_down, st0), 3)
    proj(1, 1, (2,))
    mxu("patch", patch_qkv(st0), 3)
    for b in range(NS, NB):
        proj(1, b)
        out_proj(1, b - NS)
    out_proj(1, NB - 2)
    mxu("half", mm_c(1, P - HB, HB // 2), 4)
    mxu(("C", 1, NB - 1), mm_c(1, P - HB // 2, HB // 2), 4)

    t_o = 41
    t_x = end[("A", 0, XS, 0)] - 38
    t_f = end[("A", 0, NB - 1, 0)]
    _start(g_x0 + g_qa)
    at(-12, wait, g_x0)
    at(-12, _start, g_qb)
    at(-8, _start, g_x1)
    at(-8, wait, g_qa)
    tasks.append((-8, prep_qkv(0, 0)))
    at(-4, _start, g_k)
    at(-4, wait, g_qb)
    tasks.append((-4, prep_qkv(0, 1)))
    at(-1, _start, g_v)
    at(-1, wait, g_x1)
    at(8, wait, g_k)
    spread(8, 4, [prep_qkv(1, kp) for kp in range(2)])
    at(16, _start, g_o)
    at(16, wait, g_v)
    spread(16, 4, [prep_qkv(2, kp) for kp in range(2)])
    at(t_o, wait, g_o)
    at(t_o, _start, g_f)
    at(t_x, wait, g_f)
    at(t_o, prep_wr)
    spread(t_o + 10, 16, [prep_wo(j) for j in range(4)])
    tasks += stream
    spread(t_f, end[("C", 0, NB - 1)] - 4 - t_f, [prep_ffn(n) for n in range(2 * len(FT))])

    def row_groups(b):
        return [(e, p) for p in range(b * HB, (b + 1) * HB, RL) for e in range(2)]

    for b in range(NB):
        gens = [ln_a(e, p) for e, p in row_groups(b)]
        if b < 2:
            spread((-12, 0)[b], (1, 5)[b], gens)
        else:
            last = end[("A", 0, b, 0)] - 12
            first = max(last - 28, t_x if b >= XS else t_o)
            spread(first, last - first, gens)

    def attn_layer(layer, ready, cap):
        prev = ready
        for b in range(NB):
            ready_b = max(ready, end[("A", layer, b, 2)] - 1)
            first = max(prev, ready_b)
            span = min(cap, end[("C", layer, b)] - 11 - first)
            assert span > 0
            groups = sorted(row_groups(b))
            for c, (e, p) in enumerate(groups):
                t = first + (c * span) // len(groups)
                t0 = max(t - 8, ready_b)
                tasks.append((t0, attn(e, p, 2 + t - t0)))
            prev = first + span

    def ln_c_layer(layer, groups):
        prev = 0
        for n, (ready, gens) in enumerate(groups):
            first = max(prev, ready + 1)
            later = [g[0] + 1 - first for g in groups[n + 1:n + 3]]
            span = max(1, min(32, max(later[0], later[-1] // 2))) if later else (4, 1)[layer]
            spread(first, span, gens)
            prev = first + span
            if layer == 1 and n != NB - 1:
                at(prev + 3, _start, out_copies(min(n, NB - 1)))
        return prev + 3

    attn_layer(0, 0, 30)
    racc = [jnp.zeros((8, 128), f32), jnp.zeros((8, 128), f32), 0]
    t_route = ln_c_layer(0, [(end[("C", 0, b)],
                              [ln_c(0, ((e, p), (e, p + 8)), racc) for e, p in row_groups(b)])
                             for b in range(NB)])
    tasks.append((t_route, route(0, st0)))
    assert t_route + 4 <= end["up"] - 5
    tasks.append((end["down"] + 1, patch_rows(st0)))

    attn_layer(1, end["patch"], 25)
    racc = [jnp.zeros((8, 128), f32), jnp.zeros((8, 128), f32), 0]
    cuts = [(end[("C", 1, b)], b * HB, (b + 1) * HB) for b in range(NB - 1)]
    cuts += [(end["half"], P - HB, P - HB // 2), (end[("C", 1, NB - 1)], P - HB // 2, P)]
    t_end = ln_c_layer(1, [(ready, [ln_c(1, ((0, p), (1, p)), racc) for p in range(a, b, 8)])
                           for ready, a, b in cuts])
    at(t_end, wait, [c for b in range(NB - 2) for c in out_copies(b)])
    tasks.append((t_end, route(1, st1)))
    at(t_end + 4, ffn_up, st1)
    at(t_end + 5, ffn_down, st1)
    _emit(tasks)

    new = st1["new"]
    base = [pl.multiple_of((p >> 3) << 3, 8) for _, p in st1["sel"]]
    sub = lax.broadcasted_iota(i32, (8, 128), 0)
    for n, b in enumerate(base):
        for j in range(4):
            words = out_w[j, pl.ds(b, 8), :]
            halves = []
            for h in range(2):
                t = _half(words, h)
                for c, (e, p) in enumerate(st1["sel"]):
                    t = jnp.where((sub + b) * 2 + h == p * 2 + e, _tile(new[c:c + 1], j), t)
                halves.append(t)
            patch_w[n * 4 + j] = _words(*halves)
    wait(out_copies(NB - 2) + out_copies(NB - 1))
    copies = [[pltpu.make_async_copy(
        patch.at[n * 4 + j],
        out_hbm.at[0, pl.ds(pl.multiple_of(2 * b, 16), 16), pl.ds(j * 128, 128)],
        sem_out.at[2 + n]) for j in range(4)] for n, b in enumerate(base)]
    _start(copies[0])

    @pl.when(base[0] != base[1])
    def _():
        _start(copies[1])
        wait(copies[1])

    wait(copies[0])


@jax.jit
def pallas_interleave_layers__sliding_local_dilated__moe_arch_mod__prompt_kernel(
    A_x: jax.Array,
    A_wqkv: jax.Array,
    A_wo: jax.Array,
    B_x: jax.Array,
    B_w_r: jax.Array,
    B_w_gate: jax.Array,
    B_w_up: jax.Array,
    B_w_down: jax.Array,
):
    del B_x
    V = pltpu.VMEM
    scratch = [
        V((4, S, 128), bf16), V((D, 3 * D), bf16), V((D, D), bf16), V((D,), bf16),
        V((F, D), bf16), V((F, D), bf16), V((F, D), bf16),
        V((2, D + 16, 128), i32), V((4, D + 16, 128), f32), V((12, D // 2, 128), i32), V((8, D), f32),
        V((2, 4, HALO + P, 128), f32), V((2, 4, HALO + P, 128), f32), V((2, 4, HALO + P, 128), f32),
        V((2, P, D), f32), V((2, P, D), f32), V((4, S, 128), bf16), V((2, 8, 128), f32),
        V((8, 16, 128), bf16),
        pltpu.SemaphoreType.DMA((8,)), pltpu.SemaphoreType.DMA((4,)),
        V((4, WF_0 + 6 * D, 128), bf16),
    ] + [V((4, TB, 128), bf16)] * NS
    return pl.pallas_call(
        _kernel,
        out_shape=jax.ShapeDtypeStruct((1, S, D), bf16),
        in_specs=[pl.BlockSpec(memory_space=pltpu.HBM)] * 7,
        out_specs=pl.BlockSpec(memory_space=pltpu.HBM),
        scratch_shapes=scratch,
        compiler_params=pltpu.CompilerParams(vmem_limit_bytes=100 * 1024 * 1024,
                                             disable_bounds_checks=True,
                                             disable_semaphore_checks=True),
        name="fused",
    )(A_x, A_wqkv, A_wo, B_w_r, B_w_gate.T, B_w_up.T, B_w_down)
```
